```python
import os as _os
_os.environ.setdefault("JAX_PLATFORMS", "cpu")
import jax
import jax.numpy as jnp

def _softmax(x, axis=-1):
    return jax.nn.softmax(x, axis=axis)
def _gelu(x):
    return jax.nn.gelu(x, approximate=True)
def _silu(x):
    return jax.nn.silu(x)
def _sigmoid(x):
    return jax.nn.sigmoid(x)
def _layernorm(x, axis=-1, eps=1e-5):
    m = jnp.mean(x, axis=axis, keepdims=True)
    v = jnp.var(x, axis=axis, keepdims=True)
    return (x - m) / jnp.sqrt(v + eps)
def _scatter_add(tgt, idx, src, axis=0):
    return tgt.at[idx].add(src)
def _segment_sum(src, seg, n):
    return jax.ops.segment_sum(src, seg, n)
class _Rng:
    def __init__(self, key):
        self._k = key
    def _next(self):
        self._k, sub = jax.random.split(self._k)
        return sub
    def normal(self, shape):
        return jax.random.normal(self._next(), shape, dtype=jnp.bfloat16)
    def randint(self, lo, hi, shape):
        return jax.random.randint(self._next(), shape, lo, hi, dtype=jnp.int32)
    def uniform(self, shape, lo=0.0, hi=1.0):
        return jax.random.uniform(self._next(), shape, jnp.bfloat16, lo, hi)
    def permutation(self, n):
        return jax.random.permutation(self._next(), n)


kernel_name = 'sequential_preLN__softmax_full_mha__mixer_channel_mlp__prompt'

def setup_inputs():
    _rng = _Rng(jax.random.key(int.from_bytes(__import__("os").urandom(4), "little")))
    _w = (lambda a: (lambda t: t.astype(jnp.bfloat16) if jnp.issubdtype(t.dtype, jnp.floating) else t)(jnp.asarray(a)))
    def _A_setup():
        B, S, D = 1, 2048, 1024
        return {
            "x": _w((lambda *s: _rng.normal(s) * 0.05)(B, S, D)),
            "wqkv": _w((lambda *s: _rng.normal(s) * 0.05)(D, 3 * D)),
            "wo": _w((lambda *s: _rng.normal(s) * 0.05)(D, D)),
        }
    _A_in = _A_setup()

    def _B_setup():
        B, S, D, F = 1, 2048, 1024, 3584
        return {
            "x": _w((lambda *s: _rng.normal(s) * 0.05)(B, S, D)),
            "w1": _w((lambda *s: _rng.normal(s) * 0.8)(D, F) * (D ** -0.5)),
            "b1": _w((lambda *s: _rng.normal(s) * 0.8)(F)),
            "w2": _w((lambda *s: _rng.normal(s) * 0.8)(F, D) * (F ** -0.5)),
            "b2": _w((lambda *s: _rng.normal(s) * 0.05)(D)),
        }
    _B_in = _B_setup()

    return {
        "A_x": _A_in["x"],
        "A_wqkv": _A_in["wqkv"],
        "A_wo": _A_in["wo"],
        "B_x": _B_in["x"],
        "B_w1": _B_in["w1"],
        "B_b1": _B_in["b1"],
        "B_w2": _B_in["w2"],
        "B_b2": _B_in["b2"],
    }

def reference(A_x, A_wqkv, A_wo, B_x, B_w1, B_b1, B_w2, B_b2):
    def _A_ref(x, wqkv, wo):
        B, S, D = x.shape
        H = 32; Dh = D // H
        qkv = (lambda x, *d: x.transpose(*d))((x @ wqkv).reshape(B, S, 3, H, Dh), 2, 0, 3, 1, 4)
        q, k, v = qkv[0], qkv[1], qkv[2]
        scale = Dh ** -0.5
        scores = jnp.einsum("bhqd,bhkd->bhqk", q, k) * scale
        p = _softmax(scores, axis=-1)
        o = jnp.einsum("bhqk,bhkd->bhqd", p, v)
        return (lambda x, *d: x.transpose(*d))(o, 0, 2, 1, 3).reshape(B, S, D) @ wo

    def _B_ref(x, w1, b1, w2, b2):
        y = _layernorm(x, axis=-1)
        h = _gelu(jnp.einsum("bsd,df->bsf", y, w1) + b1)
        return jnp.einsum("bsf,fd->bsd", h, w2) + b2

    x = A_x
    h = x + _A_ref(_layernorm(x, axis=-1), A_wqkv, A_wo)
    h2 = h + _B_ref(_layernorm(h, axis=-1), B_w1, B_b1, B_w2, B_b2)
    return h2
```

```python
import functools
import math

import jax
import jax.numpy as jnp
from jax import lax
import jax.experimental.pallas as pl
import jax.experimental.pallas.tpu as pltpu

_H = 32
_EPS = 1e-5
_NT = (((1,), (1,)), ((), ()))
_TN = (((0,), (0,)), ((), ()))

_TQ = 512
_TK = 128
_UNROLL = 4
_SKEW = 1
_TF = 512


def _layernorm(x):
    m = jnp.mean(x, axis=-1, keepdims=True)
    xc = x - m
    v = jnp.mean(xc * xc, axis=-1, keepdims=True)
    return xc * lax.rsqrt(v + _EPS)


def _gelu(x):
    c = math.sqrt(2.0 / math.pi)
    return 0.5 * x * (1.0 + jnp.tanh(c * (x + 0.044715 * (x * x * x))))


def _kernel(x_ref, wqkv_hbm, wo_hbm, w1_hbm, b1_ref, w2_hbm, b2_ref, o_ref,
            wqkv_s, wo_s, w1_s, w2_s, qm_s, k_s, vt_s, sA, sB, mA, mB, m8_s,
            ot_s, h_s, y_s, acc_s, sems, *, S, D, F):
    H = _H
    DH = D // H
    tq, tk, d = _TQ, _TK, _SKEW
    nq = S // tq
    nkc = S // tk
    G = D // 128
    HPG = 128 // DH
    step = pl.program_id(0)

    def weight_copies():
        return [
            pltpu.make_async_copy(wqkv_hbm, wqkv_s, sems.at[0]),
            pltpu.make_async_copy(wo_hbm, wo_s, sems.at[1]),
            pltpu.make_async_copy(w1_hbm, w1_s, sems.at[2]),
            pltpu.make_async_copy(w2_hbm, w2_s, sems.at[3]),
        ]

    @pl.when(step == 0)
    def _():
        cps = weight_copies()
        for c in cps:
            c.start()
        cps[0].wait()

    sbuf = [sA, sB]
    mbuf = [mA, mB]

    def qk_chunk(qb, h, par, kc, m8):
        g = h // HPG if isinstance(h, int) else lax.shift_right_logical(h, 2)
        qoff = qb * tq if isinstance(qb, int) else pl.multiple_of(qb * tq, tq)
        s = lax.dot_general(k_s[g, kc * tk:(kc + 1) * tk, :],
                            qm_s[h, pl.ds(qoff, tq), :], _NT,
                            preferred_element_type=jnp.float32)
        sbuf[par][kc * tk:(kc + 1) * tk, :] = s
        mc = jnp.max(s.reshape(tk // 8, 8, tq), axis=0)
        m8 = mc if m8 is None else jnp.maximum(m8, mc)
        if kc == nkc - 1:
            mbuf[par][...] = jnp.max(m8, axis=0, keepdims=True)
        return m8

    @pl.when(step < nq)
    def _():
        roff = pl.multiple_of(step * tq, tq)
        xn = _layernorm(x_ref[...].astype(jnp.float32)).astype(jnp.bfloat16)
        qscale = (DH ** -0.5) * math.log2(math.e)
        lane = lax.broadcasted_iota(jnp.int32, (tq, 128), 1)
        q = jnp.dot(xn, wqkv_s[:, 0:D], preferred_element_type=jnp.float32) * qscale
        for g in range(G):
            qg = q[:, g * 128:(g + 1) * 128]
            for hh in range(HPG):
                msk = (lane >= hh * DH) & (lane < (hh + 1) * DH)
                qm_s[g * HPG + hh, pl.ds(roff, tq), :] = jnp.where(
                    msk, qg, 0.0).astype(jnp.bfloat16)
        k = jnp.dot(xn, wqkv_s[:, D:2 * D], preferred_element_type=jnp.float32)
        for g in range(G):
            k_s[g, pl.ds(roff, tq), :] = k[:, g * 128:(g + 1) * 128].astype(jnp.bfloat16)
        v = jnp.dot(xn, wqkv_s[:, 2 * D:3 * D], preferred_element_type=jnp.float32)
        vt = v.T.astype(jnp.bfloat16)
        for blk in range(nq):
            @pl.when(step == blk)
            def _():
                for h in range(H):
                    vt_s[h, :, blk * tq:(blk + 1) * tq] = vt[h * DH:(h + 1) * DH, :]

    @pl.when(step == nq - 1)
    def _():
        m8 = None
        for kc in range(nkc):
            m8 = qk_chunk(0, 0, 0, kc, m8)
        m8 = None
        for kc in range(d):
            m8 = qk_chunk(0, 1, 1, kc, m8)
        if d:
            m8_s[...] = m8

    @pl.when(step >= nq)
    def _():
        qb = step - nq

        def body(j, c):
            h0 = j * _UNROLL
            m8 = m8_s[...] if d else None
            m_hist = []
            for u in range(_UNROLL):
                h = h0 + u
                par = u % 2
                m = jnp.broadcast_to(mbuf[par][...], (8, tq))
                acc = None
                l8 = None
                l_hist = []
                for kc in range(nkc):
                    me = m
                    if kc >= 1:
                        me = me + jnp.minimum(l_hist[kc - 1], 0.0)
                    if len(m_hist) >= 2:
                        mm = m_hist[-2]
                        me = me + jnp.where(mm == mm, 0.0, mm)
                    p = jnp.exp2(sbuf[par][kc * tk:(kc + 1) * tk, :]
                                 .reshape(tk // 8, 8, tq) - me)
                    lc = jnp.sum(p, axis=0)
                    l8 = lc if l8 is None else l8 + lc
                    l_hist.append(l8)
                    pb = p.reshape(tk, tq).astype(jnp.bfloat16)
                    tt = u * nkc + kc + nkc + d
                    un, kn = tt // nkc, tt % nkc
                    if kn == 0:
                        m8 = None
                    hn = h0 + un
                    if un < _UNROLL:
                        qbn, hn_ = qb, hn
                    else:
                        wrap = (hn >= H).astype(jnp.int32)
                        qbn = jnp.minimum(qb + wrap, nq - 1)
                        hn_ = hn - wrap * H
                    m8 = qk_chunk(qbn, hn_, un % 2, kn, m8)
                    m_hist.append(m8)
                    r = jnp.dot(vt_s[h, :, kc * tk:(kc + 1) * tk], pb,
                                preferred_element_type=jnp.float32)
                    acc = r if acc is None else acc + r
                l = jnp.sum(l8, axis=0, keepdims=True)
                ot_s[pl.ds(pl.multiple_of(h * DH, DH), DH), :] = acc * (1.0 / l)
            if d:
                m8_s[...] = m8
            return c

        lax.fori_loop(0, H // _UNROLL, body, 0)

        @pl.when(step == nq)
        def _():
            cps = weight_copies()
            for c in cps[1:]:
                c.wait()

        o = ot_s[...].T.astype(jnp.bfloat16)
        hres = x_ref[...].astype(jnp.float32) + jnp.dot(
            o, wo_s[...], preferred_element_type=jnp.float32)
        y_s[...] = _layernorm(_layernorm(hres)).astype(jnp.bfloat16)
        acc_s[...] = hres + b2_ref[...].astype(jnp.float32)

        def mlp(c, carry):
            foff = pl.multiple_of(c * _TF, _TF)
            hid = jnp.dot(y_s[...], w1_s[:, pl.ds(foff, _TF)],
                          preferred_element_type=jnp.float32)
            hid = _gelu(hid + b1_ref[:, pl.ds(foff, _TF)].astype(jnp.float32))
            acc_s[...] += jnp.dot(hid.astype(jnp.bfloat16), w2_s[pl.ds(foff, _TF), :],
                                  preferred_element_type=jnp.float32)
            return carry

        lax.fori_loop(0, F // _TF, mlp, 0)
        o_ref[...] = acc_s[...].astype(o_ref.dtype)


@jax.jit
def pallas_sequential_preLN__softmax_full_mha__mixer_channel_mlp__prompt_kernel(
    A_x: jax.Array,
    A_wqkv: jax.Array,
    A_wo: jax.Array,
    B_x: jax.Array,
    B_w1: jax.Array,
    B_b1: jax.Array,
    B_w2: jax.Array,
    B_b2: jax.Array,
):
    B, S, D = A_x.shape
    assert B == 1
    F = B_w1.shape[1]
    H, tq = _H, _TQ
    DH = D // H
    nq = S // tq
    x = A_x.reshape(S, D)
    b1 = B_b1.reshape(1, F)
    b2 = B_b2.reshape(1, D)
    bf = jnp.bfloat16
    f32 = jnp.float32

    out = pl.pallas_call(
        functools.partial(_kernel, S=S, D=D, F=F),
        grid=(2 * nq,),
        in_specs=[
            pl.BlockSpec((tq, D), lambda i: (i % nq, 0)),
            pl.BlockSpec(memory_space=pl.ANY),
            pl.BlockSpec(memory_space=pl.ANY),
            pl.BlockSpec(memory_space=pl.ANY),
            pl.BlockSpec((1, F), lambda i: (0, 0)),
            pl.BlockSpec(memory_space=pl.ANY),
            pl.BlockSpec((1, D), lambda i: (0, 0)),
        ],
        out_specs=pl.BlockSpec((tq, D), lambda i: (jnp.maximum(i - nq, 0), 0)),
        out_shape=jax.ShapeDtypeStruct((S, D), A_x.dtype),
        scratch_shapes=[
            pltpu.VMEM((D, 3 * D), bf),
            pltpu.VMEM((D, D), bf),
            pltpu.VMEM((D, F), bf),
            pltpu.VMEM((F, D), bf),
            pltpu.VMEM((H, S, 128), bf),
            pltpu.VMEM((D // 128, S, 128), bf),
            pltpu.VMEM((H, DH, S), bf),
            pltpu.VMEM((S, tq), f32),
            pltpu.VMEM((S, tq), f32),
            pltpu.VMEM((1, tq), f32),
            pltpu.VMEM((1, tq), f32),
            pltpu.VMEM((8, tq), f32),
            pltpu.VMEM((D, tq), f32),
            pltpu.VMEM((tq, D), f32),
            pltpu.VMEM((tq, D), bf),
            pltpu.VMEM((tq, D), f32),
            pltpu.SemaphoreType.DMA((4,)),
        ],
        compiler_params=pltpu.CompilerParams(
            dimension_semantics=("arbitrary",),
            vmem_limit_bytes=110 * 1024 * 1024,
        ),
    )(x, A_wqkv, A_wo, B_w1, b1, B_w2, b2)
    return out.reshape(B, S, D)
```

```python
import functools
import math

import jax
import jax.numpy as jnp
from jax import lax
import jax.experimental.pallas as pl
import jax.experimental.pallas.tpu as pltpu

_H = 32
_EPS = 1e-5

_TQ = 512
_TK = 128
_UNROLL = 8
_SKEW = 2
_TF0 = 512
_MROWS = 512
_TF = 1024
_LAG = 1
_MLAG = 2
_NC = 4
_NW0 = 3
_WOROWS = 128
_M1SPLIT = 2


def _layernorm(x):
    m = jnp.mean(x, axis=-1, keepdims=True)
    xc = x - m
    v = jnp.mean(xc * xc, axis=-1, keepdims=True)
    return xc * lax.rsqrt(v + _EPS)


def _layernorm_twice(x):
    m = jnp.mean(x, axis=-1, keepdims=True)
    xc = x - m
    v = jnp.mean(xc * xc, axis=-1, keepdims=True)
    r1 = lax.rsqrt(v + _EPS)
    r2 = lax.rsqrt(v * (r1 * r1) + _EPS)
    return xc * (r1 * r2)


def _gelu(x):
    c = math.sqrt(2.0 / math.pi)
    return 0.5 * x * (1.0 + jnp.tanh(c * (x + 0.044715 * (x * x * x))))


def _kernel(x_hbm, wqkv_hbm, wo_hbm, w1_hbm, b1_hbm, w2_hbm, b2_hbm, o_hbm,
            x_s, wqkv_s, wo_s, w1_s, w2_s, xn_s, r_s, t_s, sA, sB, mA, mB, m8_s,
            z_s, otg_s, o_s, y_s, acc_s, out_s, b1_s, b2_s, b1r_s, b2r_s,
            xsem, x1sem, w0sem, wsem, lsem, osem, *, S, D, F):
    H = _H
    DH = D // H
    tq, tk, d = _TQ, _TK, _SKEW
    nq = S // tq
    nkc = S // tk
    cpb = tq // tk
    G = D // 128
    HPG = 128 // DH
    GPI = _UNROLL // HPG
    NC = _NC
    CW = 3 * D // NC
    TPC = CW // 128
    LNR = tq // NC
    W0W = CW // _NW0
    NM = tq // _MROWS
    f32 = jnp.float32
    bf16 = jnp.bfloat16
    u32 = jnp.uint32

    def ld(x):
        return pltpu.bitcast(x, bf16)

    def st(x):
        return pltpu.bitcast(x, u32)

    def x0_copy():
        return pltpu.make_async_copy(x_hbm.at[0:tq, :], x_s.at[0:tq, :], xsem.at[0])

    def xrest_copy():
        return pltpu.make_async_copy(x_hbm.at[2 * tq:S, :], x_s.at[2 * tq:S, :],
                                     xsem.at[1])

    def x1_copy(c):
        return pltpu.make_async_copy(x_hbm.at[pl.ds(tq + c * LNR, LNR), :],
                                     x_s.at[pl.ds(tq + c * LNR, LNR), :], x1sem.at[c])

    def w0_copy(i):
        return pltpu.make_async_copy(wqkv_hbm.at[:, i * W0W:(i + 1) * W0W],
                                     wqkv_s.at[0, :, i * W0W:(i + 1) * W0W], w0sem.at[i])

    def w_copy(c):
        return pltpu.make_async_copy(wqkv_hbm.at[:, pl.ds(c * CW, CW)],
                                     wqkv_s.at[c], wsem.at[c])

    def late_copies():
        return [
            pltpu.make_async_copy(wo_hbm, wo_s, lsem.at[0]),
            pltpu.make_async_copy(w1_hbm, w1_s, lsem.at[1]),
            pltpu.make_async_copy(w2_hbm, w2_s, lsem.at[2]),
            pltpu.make_async_copy(b1_hbm, b1r_s, lsem.at[3]),
            pltpu.make_async_copy(b2_hbm, b2r_s, lsem.at[4]),
        ]

    def out_copy(qb, i):
        return pltpu.make_async_copy(
            out_s.at[pl.ds(i * _MROWS, _MROWS), :],
            o_hbm.at[pl.ds(qb * tq + i * _MROWS, _MROWS), :], osem.at[i])

    qscale = (DH ** -0.5) * math.log2(math.e)

    def ln_next(r, c, slot):
        rn = min(r + 1, nq - 1) if isinstance(r, int) else jnp.minimum(r + 1, nq - 1)
        xoff = rn * tq + c * LNR
        noff = c * (LNR // 2)
        if not isinstance(xoff, int):
            xoff = pl.multiple_of(xoff, LNR)
            noff = pl.multiple_of(noff, LNR // 2)
        xn = _layernorm(x_s[pl.ds(xoff, LNR), :].astype(f32)).astype(bf16)
        xn_s[1 - slot, pl.ds(noff, LNR // 2), :] = st(xn)

    x0_copy().start()
    w0_copy(0).start()
    otg_s[...] = jnp.zeros_like(otg_s)
    z_s[...] = jnp.zeros_like(z_s)
    x0_copy().wait()
    for i in range(1, _NW0):
        w0_copy(i).start()
    x1_copy(0).start()
    xn_s[0] = st(_layernorm(x_s[0:tq, :].astype(f32)).astype(bf16))
    assert CW <= D
    for i in range(_NW0):
        if i == _NW0 - 1:
            w_copy(1).start()
            x1_copy(1).start()
            x1_copy(0).wait()
        w0_copy(i).wait()
        res = jnp.dot(ld(xn_s[0]), wqkv_s[0, :, i * W0W:(i + 1) * W0W],
                      preferred_element_type=f32) * qscale
        resb = st(res.astype(bf16))
        for t in range(W0W // 128):
            r_s[i * (W0W // 128) + t, 0:tq // 2, :] = resb[:, t * 128:(t + 1) * 128]
    ln_next(0, 0, 0)

    def transpose_tiles(r, c):
        roff = pl.multiple_of(r * (tq // 2), tq // 2)
        for t in range(TPC):
            tile = c * TPC + t
            v = ld(r_s[tile, pl.ds(roff, tq // 2), :])
            t_s[tile, r] = st(v.T)

    def proj(it, carry):
        r = lax.shift_right_logical(it, 2)
        c = lax.rem(it, NC)

        @pl.when(r == 0)
        def _():
            w_copy(c).wait()

        @pl.when(it < NC - 1)
        def _():
            w_copy(it + 1).start()
            x1_copy(it + 1).start()

        @pl.when(it == NC - 1)
        def _():
            xrest_copy().start()

        @pl.when(r == 0)
        def _():
            x1_copy(c).wait()

        @pl.when(it == NC)
        def _():
            xrest_copy().wait()

        transpose_tiles(lax.shift_right_logical(it - 1, 2), lax.rem(it - 1, NC))

        slot = lax.rem(r, 2)
        res = jnp.dot(ld(xn_s[slot]), wqkv_s[c], preferred_element_type=f32)
        col = c * CW + lax.broadcasted_iota(jnp.int32, (1, CW), 1)
        res = res * jnp.where(col < D, qscale, 1.0)
        roff = pl.multiple_of(r * (tq // 2), tq // 2)
        resb = st(res.astype(bf16))
        for t in range(TPC):
            r_s[c * TPC + t, pl.ds(roff, tq // 2), :] = resb[:, t * 128:(t + 1) * 128]
        ln_next(r, c, slot)
        return carry

    lax.fori_loop(1, nq * NC, proj, 0)

    for cp in late_copies():
        cp.start()

    sbuf = [sA, sB]
    mbuf = [mA, mB]

    def qk_chunk(qb, h, hh, par, kc, m8):
        g = h // HPG if isinstance(h, int) else lax.shift_right_logical(h, 2)
        kk = ld(r_s[G + g, kc * tk // 2:(kc + 1) * tk // 2, :])
        parts = []
        if hh > 0:
            parts.append(jnp.zeros((hh * DH // 2, tq), u32))
        parts.append(t_s[g, qb, hh * DH // 2:(hh + 1) * DH // 2, :])
        if hh < HPG - 1:
            parts.append(jnp.zeros(((HPG - 1 - hh) * DH // 2, tq), u32))
        qm = ld(jnp.concatenate(parts, axis=0))
        s = jnp.dot(kk, qm, preferred_element_type=f32)
        sbuf[par][kc * tk:(kc + 1) * tk, :] = s
        mc = jnp.max(s.reshape(tk // 8, 8, tq), axis=0)
        m8 = mc if m8 is None else jnp.maximum(m8, mc)
        if kc == nkc - 1:
            mbuf[par][...] = jnp.max(m8, axis=0, keepdims=True)
        return m8

    transpose_tiles(nq - 1, NC - 1)
    m8 = None
    for kc in range(nkc):
        m8 = qk_chunk(0, 0, 0, 0, kc, m8)
    m8 = None
    for kc in range(d):
        m8 = qk_chunk(0, 1, 1, 1, kc, m8)
    if d:
        m8_s[...] = m8

    def flush_o(jprev):
        for gi in range(GPI):
            o_s[jprev * GPI + gi] = st(
                otg_s[gi * 128:(gi + 1) * 128, :].T.astype(bf16))

    def block(qb, carry):
        niter = H // _UNROLL

        def body(j, c):
            h0 = j * _UNROLL
            flush_o(jnp.maximum(j - 1, 0))
            m8 = m8_s[...] if d else None
            m_hist = []
            for u in range(_UNROLL):
                par = u % 2
                g = j * GPI + u // HPG
                hh = u % HPG
                m = jnp.broadcast_to(mbuf[par][...], (8, tq))
                acc = z_s[...]
                l8 = None
                l_hist = []
                for kc in range(nkc):
                    me = m
                    if _LAG and kc >= _LAG:
                        me = me + jnp.minimum(l_hist[kc - _LAG], 0.0)
                    if _MLAG and len(m_hist) >= _MLAG:
                        mm = m_hist[-_MLAG]
                        me = me + jnp.where(mm == mm, 0.0, mm)
                    p = jnp.exp2(sbuf[par][kc * tk:(kc + 1) * tk, :]
                                 .reshape(tk // 8, 8, tq) - me)
                    lc = jnp.sum(p, axis=0)
                    l8 = lc if l8 is None else l8 + lc
                    l_hist.append(l8)
                    pb = p.reshape(tk, tq).astype(bf16)
                    tt = u * nkc + kc + nkc + d
                    un, kn = tt // nkc, tt % nkc
                    if kn == 0:
                        m8 = None
                    hn = h0 + un
                    if un < _UNROLL:
                        qbn, hn_ = qb, hn
                    else:
                        wrap = (hn >= H).astype(jnp.int32)
                        qbn = jnp.minimum(qb + wrap, nq - 1)
                        hn_ = hn - wrap * H
                    m8 = qk_chunk(qbn, hn_, un % HPG, un % 2, kn, m8)
                    m_hist.append(m8)
                    vt = ld(t_s[2 * G + g, kc // cpb, hh * DH // 2:(hh + 1) * DH // 2,
                                (kc % cpb) * tk:(kc % cpb + 1) * tk])
                    acc = acc + jnp.dot(vt, pb, preferred_element_type=f32)
                l = jnp.sum(l8, axis=0, keepdims=True)
                otg_s[u * DH:(u + 1) * DH, :] = acc * (1.0 / l)
            if d:
                m8_s[...] = m8
            return c

        lax.fori_loop(0, niter, body, 0)

        @pl.when(qb == 0)
        def _():
            for cp in late_copies():
                cp.wait()
            b1_s[...] = b1r_s[...].astype(f32).reshape(1, F)
            b2_s[...] = b2r_s[...].astype(f32).reshape(1, D)

        @pl.when(qb > 0)
        def _():
            for i in range(NM):
                out_copy(qb - 1, i).wait()

        flush_o(niter - 1)
        xoff = pl.multiple_of(qb * tq, tq)
        for r0 in range(0, tq, _WOROWS):
            r1 = r0 + _WOROWS
            o = jnp.concatenate([ld(o_s[g, r0 // 2:r1 // 2, :]) for g in range(G)], axis=1)
            hres = x_s[pl.ds(xoff + r0, _WOROWS), :].astype(f32) + jnp.dot(
                o, wo_s[...], preferred_element_type=f32)
            y_s[r0 // 2:r1 // 2, :] = st(_layernorm_twice(hres).astype(bf16))
            acc_s[r0:r1, :] = hres

        w1c = w1_s[:, 0:_TF0]
        b1c = b1_s[:, 0:_TF0]
        rows = tq // _M1SPLIT
        hids = []
        for i in range(_M1SPLIT):
            hid = jnp.dot(ld(y_s[i * rows // 2:(i + 1) * rows // 2, :]), w1c,
                          preferred_element_type=f32)
            hids.append(_gelu(hid + b1c).astype(bf16))
        hid = hids[0] if _M1SPLIT == 1 else jnp.concatenate(hids, axis=0)
        acc_s[...] = (acc_s[...] + jnp.dot(hid, w2_s[0:_TF0, :],
                                           preferred_element_type=f32)) + b2_s[...]

        def mlp(c, carry):
            foff = pl.multiple_of(_TF0 + c * _TF, 128)
            hid = jnp.dot(ld(y_s[...]), w1_s[:, pl.ds(foff, _TF)],
                          preferred_element_type=f32)
            hid = _gelu(hid + b1_s[:, pl.ds(foff, _TF)]).astype(bf16)
            a = acc_s[...] + jnp.dot(hid, w2_s[pl.ds(foff, _TF), :],
                                     preferred_element_type=f32)
            acc_s[...] = a
            out_s[...] = a.astype(out_s.dtype)
            return carry

        lax.fori_loop(0, (F - _TF0) // _TF, mlp, 0)
        for i in range(NM):
            out_copy(qb, i).start()
        return carry

    lax.fori_loop(0, nq, block, 0)
    for i in range(NM):
        out_copy(nq - 1, i).wait()


@jax.jit
def pallas_sequential_preLN__softmax_full_mha__mixer_channel_mlp__prompt_kernel(
    A_x: jax.Array,
    A_wqkv: jax.Array,
    A_wo: jax.Array,
    B_x: jax.Array,
    B_w1: jax.Array,
    B_b1: jax.Array,
    B_w2: jax.Array,
    B_b2: jax.Array,
):
    B, S, D = A_x.shape
    assert B == 1
    F = B_w1.shape[1]
    H, tq = _H, _TQ
    DH = D // H
    nq = S // tq
    G = D // 128
    x = A_x.reshape(S, D)
    bf = jnp.bfloat16
    f32 = jnp.float32
    u32 = jnp.uint32
    hbm = pl.BlockSpec(memory_space=pl.ANY)

    out = pl.pallas_call(
        functools.partial(_kernel, S=S, D=D, F=F),
        in_specs=[hbm] * 7,
        out_specs=hbm,
        out_shape=jax.ShapeDtypeStruct((S, D), A_x.dtype),
        scratch_shapes=[
            pltpu.VMEM((S, D), bf),
            pltpu.VMEM((_NC, D, 3 * D // _NC), bf),
            pltpu.VMEM((D, D), bf),
            pltpu.VMEM((D, F), bf),
            pltpu.VMEM((F, D), bf),
            pltpu.VMEM((2, tq // 2, D), u32),
            pltpu.VMEM((3 * G, S // 2, 128), u32),
            pltpu.VMEM((3 * G, nq, 64, tq), u32),
            pltpu.VMEM((S, tq), f32),
            pltpu.VMEM((S, tq), f32),
            pltpu.VMEM((1, tq), f32),
            pltpu.VMEM((1, tq), f32),
            pltpu.VMEM((8, tq), f32),
            pltpu.VMEM((DH, tq), f32),
            pltpu.VMEM((_UNROLL * DH, tq), f32),
            pltpu.VMEM((G, tq // 2, 128), u32),
            pltpu.VMEM((tq // 2, D), u32),
            pltpu.VMEM((tq, D), f32),
            pltpu.VMEM((tq, D), bf),
            pltpu.VMEM((1, F), f32),
            pltpu.VMEM((1, D), f32),
            pltpu.VMEM((F,), bf),
            pltpu.VMEM((D,), bf),
            pltpu.SemaphoreType.DMA((2,)),
            pltpu.SemaphoreType.DMA((_NC,)),
            pltpu.SemaphoreType.DMA((_NW0,)),
            pltpu.SemaphoreType.DMA((_NC,)),
            pltpu.SemaphoreType.DMA((5,)),
            pltpu.SemaphoreType.DMA((tq // _MROWS,)),
        ],
        compiler_params=pltpu.CompilerParams(
            vmem_limit_bytes=110 * 1024 * 1024,
        ),
    )(x, A_wqkv, A_wo, B_w1, B_b1, B_w2, B_b2)
    return out.reshape(B, S, D)
```

```python
import functools
import math

import jax
import jax.numpy as jnp
from jax import lax
import jax.experimental.pallas as pl
import jax.experimental.pallas.tpu as pltpu

_H = 32
_EPS = 1e-5

_TQ = 512
_TK = 128
_UNROLL = 8
_SKEW = 2
_LAG = 1
_MLAG = 2
_NC = 4
_NW0 = 3
_PSPLIT = 384
_WOROWS = 128
_WOLAG = 3
_TF0 = 512
_TF = 1024


def _layernorm(x):
    m = jnp.mean(x, axis=-1, keepdims=True)
    xc = x - m
    v = jnp.mean(xc * xc, axis=-1, keepdims=True)
    return xc * lax.rsqrt(v + _EPS)


def _layernorm_twice(x):
    m = jnp.mean(x, axis=-1, keepdims=True)
    xc = x - m
    v = jnp.mean(xc * xc, axis=-1, keepdims=True)
    r1 = lax.rsqrt(v + _EPS)
    m2 = r1 * jnp.mean(xc, axis=-1, keepdims=True)
    v2 = jnp.maximum(v * (r1 * r1) - m2 * m2, 0.0)
    r2 = lax.rsqrt(v2 + _EPS)
    return xc * (r1 * r2) - m2 * r2


def _gelu(x):
    c = math.sqrt(2.0 / math.pi)
    return 0.5 * x * (1.0 + jnp.tanh(c * (x + 0.044715 * (x * x * x))))


def _kernel(x_hbm, wqkv_hbm, wo_hbm, w1_hbm, b1_hbm, w2_hbm, b2_hbm, o_hbm,
            x_s, wqkv_s, wo_s, w1_s, w2_s, xn_s, r_s, t_s, stg_s, sA, sB, mA, mB,
            m8_s, z_s, otg_s, o_s, y_s, acc_s, out_s, b1_s, b2_s, b1r_s, b2r_s,
            xsem, x1sem, w0sem, wsem, lsem, osem, *, S, D, F):
    H = _H
    DH = D // H
    tq, tk, d = _TQ, _TK, _SKEW
    nq = S // tq
    nkc = S // tk
    cpb = tq // tk
    G = D // 128
    HPG = 128 // DH
    GPI = _UNROLL // HPG
    NC = _NC
    CW = 3 * D // NC
    TPC = CW // 128
    LNR = tq // NC
    W0W = CW // _NW0
    hq = tq // 2
    f32 = jnp.float32
    bf16 = jnp.bfloat16
    u32 = jnp.uint32
    assert HPG == 4 and NC == 4 and CW <= D and nq >= 3

    def ld(x):
        return pltpu.bitcast(x, bf16)

    def st(x):
        return pltpu.bitcast(x, u32)

    def x0_copy(i):
        rows = slice(i * hq, (i + 1) * hq)
        return pltpu.make_async_copy(x_hbm.at[rows, :], x_s.at[rows, :], xsem.at[i])

    def x1_copy(c):
        return pltpu.make_async_copy(x_hbm.at[pl.ds(tq + c * LNR, LNR), :],
                                     x_s.at[pl.ds(tq + c * LNR, LNR), :], x1sem.at[c])

    def xrest_copy():
        return pltpu.make_async_copy(x_hbm.at[2 * tq:S, :], x_s.at[2 * tq:S, :],
                                     xsem.at[2])

    def w0_copy(i):
        return pltpu.make_async_copy(wqkv_hbm.at[:, i * W0W:(i + 1) * W0W],
                                     wqkv_s.at[0, :, i * W0W:(i + 1) * W0W], w0sem.at[i])

    def w_copy(c):
        return pltpu.make_async_copy(wqkv_hbm.at[:, pl.ds(c * CW, CW)],
                                     wqkv_s.at[c], wsem.at[c])

    def late_copies():
        return [
            pltpu.make_async_copy(wo_hbm, wo_s, lsem.at[0]),
            pltpu.make_async_copy(w1_hbm, w1_s, lsem.at[1]),
            pltpu.make_async_copy(w2_hbm, w2_s, lsem.at[2]),
            pltpu.make_async_copy(b1_hbm, b1r_s, lsem.at[3]),
            pltpu.make_async_copy(b2_hbm, b2r_s, lsem.at[4]),
        ]

    def out_copy(qb):
        return pltpu.make_async_copy(out_s, o_hbm.at[pl.ds(qb * tq, tq), :], osem.at[0])

    qscale = (DH ** -0.5) * math.log2(math.e)

    x0_copy(0).start()
    w0_copy(0).start()
    x0_copy(1).start()
    otg_s[...] = jnp.zeros_like(otg_s)
    z_s[...] = jnp.zeros_like(z_s)
    x0_copy(0).wait()
    xn_s[0, 0:hq // 2, :] = st(_layernorm(x_s[0:hq, :].astype(f32)).astype(bf16))
    x0_copy(1).wait()
    for i in range(1, _NW0):
        w0_copy(i).start()
    x1_copy(0).start()
    for i in range(_NW0):
        if i == 1:
            w_copy(1).start()
            x1_copy(1).start()
        if i == _NW0 - 1:
            x1_copy(0).wait()
        w0_copy(i).wait()
        wp = wqkv_s[0, :, i * W0W:(i + 1) * W0W]
        if i == 0:
            ra = jnp.dot(ld(xn_s[0, 0:hq // 2, :]), wp, preferred_element_type=f32)
            xn_s[0, hq // 2:hq, :] = st(
                _layernorm(x_s[hq:tq, :].astype(f32)).astype(bf16))
            rb = jnp.dot(ld(xn_s[0, hq // 2:hq, :]), wp, preferred_element_type=f32)
            res = jnp.concatenate([ra, rb], axis=0) * qscale
        else:
            res = jnp.dot(ld(xn_s[0]), wp, preferred_element_type=f32) * qscale
        resb = st(res.astype(bf16))
        for t in range(W0W // 128):
            stg_s[i * (W0W // 128) + t] = resb[:, t * 128:(t + 1) * 128]
    xn_s[1, 0:LNR // 2, :] = st(_layernorm(x_s[tq:tq + LNR, :].astype(f32)).astype(bf16))

    def transpose_tiles(r, c):
        for t in range(TPC):
            t_s[c * TPC + t, r] = st(ld(stg_s[t]).T)

    def proj(it, carry):
        r = lax.shift_right_logical(it, 2)
        c = lax.rem(it, NC)

        @pl.when(it < NC)
        def _():
            w_copy(c).wait()

        for k in range(2, NC):
            @pl.when(it == k - 1)
            def _():
                w_copy(k).start()
                x1_copy(k).start()

        @pl.when(it == NC - 1)
        def _():
            xrest_copy().start()

        @pl.when(it < NC)
        def _():
            x1_copy(c).wait()

        @pl.when(it == NC)
        def _():
            xrest_copy().wait()

        transpose_tiles(lax.shift_right_logical(it - 1, 2), lax.rem(it - 1, NC))

        slot = lax.rem(r, 2)
        rn = jnp.minimum(r + 1, nq - 1)
        xoff = pl.multiple_of(rn * tq + c * LNR, LNR)
        xnb = st(_layernorm(x_s[pl.ds(xoff, LNR), :].astype(f32)).astype(bf16))
        t = xnb.reshape(LNR // 16, 8, D)
        z = t[0]
        for i in range(1, LNR // 16):
            z = z & t[i]
        z = z & pltpu.bitcast(jnp.concatenate([z_s[0:8, :]] * (D // tq), axis=1), u32)
        lhs = xn_s[slot]
        lhs2 = jnp.concatenate([lhs[0:8] | z, lhs[8:]], axis=0)
        sp = _PSPLIT
        res = jnp.concatenate(
            [jnp.dot(ld(lhs), wqkv_s[c, :, 0:sp], preferred_element_type=f32),
             jnp.dot(ld(lhs2), wqkv_s[c, :, sp:CW], preferred_element_type=f32)], axis=1)
        col = c * CW + lax.broadcasted_iota(jnp.int32, (1, CW), 1)
        res = res * jnp.where(col < D, qscale, 1.0)
        roff = pl.multiple_of(r * hq, hq)
        resb = st(res.astype(bf16))
        for t_ in range(TPC):
            r_s[c * TPC + t_, pl.ds(roff, hq), :] = resb[:, t_ * 128:(t_ + 1) * 128]
            stg_s[t_] = resb[:, t_ * 128:(t_ + 1) * 128]
        noff = pl.multiple_of(c * (LNR // 2), LNR // 2)
        xn_s[1 - slot, pl.ds(noff, LNR // 2), :] = xnb
        return carry

    lax.fori_loop(1, nq * NC, proj, 0)

    for cp in late_copies():
        cp.start()

    sbuf = [sA, sB]
    mbuf = [mA, mB]

    def qk_chunk(qb, h, hh, par, kc, m8):
        g = h // HPG if isinstance(h, int) else lax.shift_right_logical(h, 2)
        kk = ld(r_s[G + g, kc * tk // 2:(kc + 1) * tk // 2, :])
        parts = []
        if hh > 0:
            parts.append(jnp.zeros((hh * DH // 2, tq), u32))
        parts.append(t_s[g, qb, hh * DH // 2:(hh + 1) * DH // 2, :])
        if hh < HPG - 1:
            parts.append(jnp.zeros(((HPG - 1 - hh) * DH // 2, tq), u32))
        qm = ld(jnp.concatenate(parts, axis=0))
        s = jnp.dot(kk, qm, preferred_element_type=f32)
        sbuf[par][kc * tk:(kc + 1) * tk, :] = s
        mc = jnp.max(s.reshape(tk // 8, 8, tq), axis=0)
        m8 = mc if m8 is None else jnp.maximum(m8, mc)
        if kc == nkc - 1:
            mbuf[par][...] = jnp.max(m8, axis=0, keepdims=True)
        return m8

    transpose_tiles(nq - 1, NC - 1)
    m8 = None
    for kc in range(nkc):
        m8 = qk_chunk(0, 0, 0, 0, kc, m8)
    m8 = None
    for kc in range(d):
        m8 = qk_chunk(0, 1, 1, 1, kc, m8)
    m8_s[...] = m8

    def flush_o(jprev):
        for gi in range(GPI):
            o_s[jprev * GPI + gi] = st(
                otg_s[gi * 128:(gi + 1) * 128, :].T.astype(bf16))

    def block(qb, carry):
        niter = H // _UNROLL

        def body(j, c):
            h0 = j * _UNROLL
            flush_o(jnp.maximum(j - 1, 0))
            m8 = m8_s[...]
            m_hist = []
            for u in range(_UNROLL):
                par = u % 2
                g = j * GPI + u // HPG
                hh = u % HPG
                m = jnp.broadcast_to(mbuf[par][...], (8, tq))
                acc = z_s[...]
                l8 = None
                l_hist = []
                for kc in range(nkc):
                    me = m
                    if kc >= _LAG:
                        me = me + jnp.minimum(l_hist[kc - _LAG], 0.0)
                    if len(m_hist) >= _MLAG:
                        mm = m_hist[-_MLAG]
                        me = me + jnp.where(mm == mm, 0.0, mm)
                    p = jnp.exp2(sbuf[par][kc * tk:(kc + 1) * tk, :]
                                 .reshape(tk // 8, 8, tq) - me)
                    lc = jnp.sum(p, axis=0)
                    l8 = lc if l8 is None else l8 + lc
                    l_hist.append(l8)
                    pb = p.reshape(tk, tq).astype(bf16)
                    tt = u * nkc + kc + nkc + d
                    un, kn = tt // nkc, tt % nkc
                    if kn == 0:
                        m8 = None
                    hn = h0 + un
                    if un < _UNROLL:
                        qbn, hn_ = qb, hn
                    else:
                        wrap = (hn >= H).astype(jnp.int32)
                        qbn = jnp.minimum(qb + wrap, nq - 1)
                        hn_ = hn - wrap * H
                    m8 = qk_chunk(qbn, hn_, un % HPG, un % 2, kn, m8)
                    m_hist.append(m8)
                    vt = ld(t_s[2 * G + g, kc // cpb, hh * DH // 2:(hh + 1) * DH // 2,
                                (kc % cpb) * tk:(kc % cpb + 1) * tk])
                    acc = acc + jnp.dot(vt, pb, preferred_element_type=f32)
                l = jnp.sum(l8, axis=0, keepdims=True)
                otg_s[u * DH:(u + 1) * DH, :] = acc * (1.0 / l)
            m8_s[...] = m8
            return c

        lax.fori_loop(0, niter, body, 0)

        @pl.when(qb == 0)
        def _():
            for cp in late_copies():
                cp.wait()
            b1_s[...] = b1r_s[...].astype(f32).reshape(1, F)
            b2_s[...] = b2r_s[...].astype(f32).reshape(1, D)

        @pl.when(qb > 0)
        def _():
            out_copy(qb - 1).wait()

        flush_o(niter - 1)
        xoff = pl.multiple_of(qb * tq, tq)
        w1c = w1_s[:, 0:_TF0]
        b1c = b1_s[:, 0:_TF0]
        npc = tq // _WOROWS
        hids = []

        def wo_piece(p):
            r0, r1 = p * _WOROWS, (p + 1) * _WOROWS
            o = jnp.concatenate([ld(o_s[g, r0 // 2:r1 // 2, :]) for g in range(G)], axis=1)
            hres = x_s[pl.ds(xoff + r0, _WOROWS), :].astype(f32) + jnp.dot(
                o, wo_s[...], preferred_element_type=f32)
            y_s[r0 // 2:r1 // 2, :] = st(_layernorm_twice(hres).astype(bf16))
            acc_s[r0:r1, :] = hres

        def m1_piece(p):
            r0, r1 = p * _WOROWS, (p + 1) * _WOROWS
            hid = jnp.dot(ld(y_s[r0 // 2:r1 // 2, :]), w1c, preferred_element_type=f32)
            hids.append(_gelu(hid + b1c).astype(bf16))

        for p in range(npc + _WOLAG):
            if p < npc:
                wo_piece(p)
            if p >= _WOLAG:
                m1_piece(p - _WOLAG)
        hid = jnp.concatenate(hids, axis=0)
        acc_s[...] = (acc_s[...] + jnp.dot(hid, w2_s[0:_TF0, :],
                                           preferred_element_type=f32)) + b2_s[...]

        def mlp(c, carry):
            foff = pl.multiple_of(_TF0 + c * _TF, 128)
            hid = jnp.dot(ld(y_s[...]), w1_s[:, pl.ds(foff, _TF)],
                          preferred_element_type=f32)
            hid = _gelu(hid + b1_s[:, pl.ds(foff, _TF)]).astype(bf16)
            a = acc_s[...] + jnp.dot(hid, w2_s[pl.ds(foff, _TF), :],
                                     preferred_element_type=f32)
            acc_s[...] = a
            out_s[...] = a.astype(out_s.dtype)
            return carry

        lax.fori_loop(0, (F - _TF0) // _TF, mlp, 0)
        out_copy(qb).start()
        return carry

    lax.fori_loop(0, nq, block, 0)
    out_copy(nq - 1).wait()


@jax.jit
def pallas_sequential_preLN__softmax_full_mha__mixer_channel_mlp__prompt_kernel(
    A_x: jax.Array,
    A_wqkv: jax.Array,
    A_wo: jax.Array,
    B_x: jax.Array,
    B_w1: jax.Array,
    B_b1: jax.Array,
    B_w2: jax.Array,
    B_b2: jax.Array,
):
    B, S, D = A_x.shape
    assert B == 1
    F = B_w1.shape[1]
    H, tq = _H, _TQ
    DH = D // H
    nq = S // tq
    G = D // 128
    assert S % tq == 0 and D % tq == 0 and (F - _TF0) % _TF == 0 and F > _TF0
    x = A_x.reshape(S, D)
    bf = jnp.bfloat16
    f32 = jnp.float32
    u32 = jnp.uint32
    hbm = pl.BlockSpec(memory_space=pl.ANY)

    out = pl.pallas_call(
        functools.partial(_kernel, S=S, D=D, F=F),
        in_specs=[hbm] * 7,
        out_specs=hbm,
        out_shape=jax.ShapeDtypeStruct((S, D), A_x.dtype),
        scratch_shapes=[
            pltpu.VMEM((S, D), bf),
            pltpu.VMEM((_NC, D, 3 * D // _NC), bf),
            pltpu.VMEM((D, D), bf),
            pltpu.VMEM((D, F), bf),
            pltpu.VMEM((F, D), bf),
            pltpu.VMEM((2, tq // 2, D), u32),
            pltpu.VMEM((3 * G, S // 2, 128), u32),
            pltpu.VMEM((3 * G, nq, 64, tq), u32),
            pltpu.VMEM((3 * D // _NC // 128, tq // 2, 128), u32),
            pltpu.VMEM((S, tq), f32),
            pltpu.VMEM((S, tq), f32),
            pltpu.VMEM((1, tq), f32),
            pltpu.VMEM((1, tq), f32),
            pltpu.VMEM((8, tq), f32),
            pltpu.VMEM((DH, tq), f32),
            pltpu.VMEM((_UNROLL * DH, tq), f32),
            pltpu.VMEM((G, tq // 2, 128), u32),
            pltpu.VMEM((tq // 2, D), u32),
            pltpu.VMEM((tq, D), f32),
            pltpu.VMEM((tq, D), bf),
            pltpu.VMEM((1, F), f32),
            pltpu.VMEM((1, D), f32),
            pltpu.VMEM((F,), bf),
            pltpu.VMEM((D,), bf),
            pltpu.SemaphoreType.DMA((3,)),
            pltpu.SemaphoreType.DMA((_NC,)),
            pltpu.SemaphoreType.DMA((_NW0,)),
            pltpu.SemaphoreType.DMA((_NC,)),
            pltpu.SemaphoreType.DMA((5,)),
            pltpu.SemaphoreType.DMA((1,)),
        ],
        compiler_params=pltpu.CompilerParams(
            vmem_limit_bytes=110 * 1024 * 1024,
        ),
    )(x, A_wqkv, A_wo, B_w1, B_b1, B_w2, B_b2)
    return out.reshape(B, S, D)
```

```python
import functools
import math

import jax
import jax.numpy as jnp
from jax import lax
import jax.experimental.pallas as pl
import jax.experimental.pallas.tpu as pltpu

_H = 32
_EPS = 1e-5

_TQ = 512
_TK = 128
_UNROLL = 8
_SKEW = 2
_MLAG = 2
_NC = 4
_NW0 = 3
_PSPLIT = 384
_WOROWS = 128
_WOLAG = 3
_TF0 = 512
_TF = 1024


def _layernorm(x):
    m = jnp.mean(x, axis=-1, keepdims=True)
    xc = x - m
    v = jnp.mean(xc * xc, axis=-1, keepdims=True)
    return xc * lax.rsqrt(v + _EPS)


def _layernorm_twice(x):
    m = jnp.mean(x, axis=-1, keepdims=True)
    xc = x - m
    v = jnp.mean(xc * xc, axis=-1, keepdims=True)
    r1 = lax.rsqrt(v + _EPS)
    m2 = r1 * jnp.mean(xc, axis=-1, keepdims=True)
    v2 = jnp.maximum(v * (r1 * r1) - m2 * m2, 0.0)
    r2 = lax.rsqrt(v2 + _EPS)
    return xc * (r1 * r2) - m2 * r2


def _gelu(x):
    c = math.sqrt(2.0 / math.pi)
    return 0.5 * x * (1.0 + jnp.tanh(c * (x + 0.044715 * (x * x * x))))


def _kernel(x_hbm, wqkv_hbm, wo_hbm, w1_hbm, b1_hbm, w2_hbm, b2_hbm, o_hbm,
            x_s, wqkv_s, wo_s, w1_s, w2_s, xn_s, r_s, t_s, stg_s, sA, sB, mA, mB,
            m8_s, z_s, otg_s, o_s, y_s, acc_s, out_s, b1_s, b2_s, b1r_s, b2r_s,
            xsem, x1sem, w0sem, wsem, lsem, osem, *, S, D, F):
    H = _H
    DH = D // H
    tq, tk, d = _TQ, _TK, _SKEW
    nq = S // tq
    nkc = S // tk
    cpb = tq // tk
    G = D // 128
    HPG = 128 // DH
    GPI = _UNROLL // HPG
    NC = _NC
    CW = 3 * D // NC
    TPC = CW // 128
    LNR = tq // NC
    W0W = CW // _NW0
    hq = tq // 2
    f32 = jnp.float32
    bf16 = jnp.bfloat16
    u32 = jnp.uint32
    assert HPG == 4 and NC == 4 and CW <= D and nq >= 3

    def ld(x):
        return pltpu.bitcast(x, bf16)

    def st(x):
        return pltpu.bitcast(x, u32)

    def x0_copy(i):
        rows = slice(i * hq, (i + 1) * hq)
        return pltpu.make_async_copy(x_hbm.at[rows, :], x_s.at[rows, :], xsem.at[i])

    def x1_copy(c):
        return pltpu.make_async_copy(x_hbm.at[pl.ds(tq + c * LNR, LNR), :],
                                     x_s.at[pl.ds(tq + c * LNR, LNR), :], x1sem.at[c])

    def xrest_copy():
        return pltpu.make_async_copy(x_hbm.at[2 * tq:S, :], x_s.at[2 * tq:S, :],
                                     xsem.at[2])

    def w0_copy(i):
        return pltpu.make_async_copy(wqkv_hbm.at[:, i * W0W:(i + 1) * W0W],
                                     wqkv_s.at[0, :, i * W0W:(i + 1) * W0W], w0sem.at[i])

    def w_copy(c):
        return pltpu.make_async_copy(wqkv_hbm.at[:, pl.ds(c * CW, CW)],
                                     wqkv_s.at[c], wsem.at[c])

    def late_copies():
        return [
            pltpu.make_async_copy(wo_hbm, wo_s, lsem.at[0]),
            pltpu.make_async_copy(w1_hbm, w1_s, lsem.at[1]),
            pltpu.make_async_copy(w2_hbm, w2_s, lsem.at[2]),
            pltpu.make_async_copy(b1_hbm, b1r_s, lsem.at[3]),
            pltpu.make_async_copy(b2_hbm, b2r_s, lsem.at[4]),
        ]

    def out_copy(qb):
        return pltpu.make_async_copy(out_s, o_hbm.at[pl.ds(qb * tq, tq), :], osem.at[0])

    qscale = (DH ** -0.5) * math.log2(math.e)

    x0_copy(0).start()
    w0_copy(0).start()
    x0_copy(1).start()
    otg_s[...] = jnp.zeros_like(otg_s)
    z_s[...] = jnp.zeros_like(z_s)
    x0_copy(0).wait()
    xn_s[0, 0:hq // 2, :] = st(_layernorm(x_s[0:hq, :].astype(f32)).astype(bf16))
    x0_copy(1).wait()
    for i in range(1, _NW0):
        w0_copy(i).start()
    x1_copy(0).start()
    for i in range(_NW0):
        if i == 1:
            w_copy(1).start()
            x1_copy(1).start()
        if i == _NW0 - 1:
            x1_copy(0).wait()
        w0_copy(i).wait()
        wp = wqkv_s[0, :, i * W0W:(i + 1) * W0W]
        if i == 0:
            ra = jnp.dot(ld(xn_s[0, 0:hq // 2, :]), wp, preferred_element_type=f32)
            xn_s[0, hq // 2:hq, :] = st(
                _layernorm(x_s[hq:tq, :].astype(f32)).astype(bf16))
            rb = jnp.dot(ld(xn_s[0, hq // 2:hq, :]), wp, preferred_element_type=f32)
            res = jnp.concatenate([ra, rb], axis=0) * qscale
        else:
            res = jnp.dot(ld(xn_s[0]), wp, preferred_element_type=f32) * qscale
        resb = st(res.astype(bf16))
        for t in range(W0W // 128):
            stg_s[i * (W0W // 128) + t] = resb[:, t * 128:(t + 1) * 128]
    xn_s[1, 0:LNR // 2, :] = st(_layernorm(x_s[tq:tq + LNR, :].astype(f32)).astype(bf16))

    def transpose_tiles(r, c):
        for t in range(TPC):
            t_s[c * TPC + t, r] = st(ld(stg_s[t]).T)

    def proj(it, carry):
        r = lax.shift_right_logical(it, 2)
        c = lax.rem(it, NC)

        @pl.when(it < NC)
        def _():
            w_copy(c).wait()

        for k in range(2, NC):
            @pl.when(it == k - 1)
            def _():
                w_copy(k).start()
                x1_copy(k).start()

        @pl.when(it == NC - 1)
        def _():
            xrest_copy().start()

        @pl.when(it < NC)
        def _():
            x1_copy(c).wait()

        @pl.when(it == NC)
        def _():
            xrest_copy().wait()

        transpose_tiles(lax.shift_right_logical(it - 1, 2), lax.rem(it - 1, NC))

        slot = lax.rem(r, 2)
        rn = jnp.minimum(r + 1, nq - 1)
        xoff = pl.multiple_of(rn * tq + c * LNR, LNR)
        xnb = st(_layernorm(x_s[pl.ds(xoff, LNR), :].astype(f32)).astype(bf16))
        t = xnb.reshape(LNR // 16, 8, D)
        z = t[0]
        for i in range(1, LNR // 16):
            z = z & t[i]
        z = z & pltpu.bitcast(jnp.concatenate([z_s[0:8, :]] * (D // tq), axis=1), u32)
        lhs = xn_s[slot]
        lhs2 = jnp.concatenate([lhs[0:8] | z, lhs[8:]], axis=0)
        sp = _PSPLIT
        res = jnp.concatenate(
            [jnp.dot(ld(lhs), wqkv_s[c, :, 0:sp], preferred_element_type=f32),
             jnp.dot(ld(lhs2), wqkv_s[c, :, sp:CW], preferred_element_type=f32)], axis=1)
        col = c * CW + lax.broadcasted_iota(jnp.int32, (1, CW), 1)
        res = res * jnp.where(col < D, qscale, 1.0)
        roff = pl.multiple_of(r * hq, hq)
        resb = st(res.astype(bf16))
        for t_ in range(TPC):
            r_s[c * TPC + t_, pl.ds(roff, hq), :] = resb[:, t_ * 128:(t_ + 1) * 128]
            stg_s[t_] = resb[:, t_ * 128:(t_ + 1) * 128]
        noff = pl.multiple_of(c * (LNR // 2), LNR // 2)
        xn_s[1 - slot, pl.ds(noff, LNR // 2), :] = xnb
        return carry

    lax.fori_loop(1, nq * NC, proj, 0)

    for cp in late_copies():
        cp.start()

    sbuf = [sA, sB]
    mbuf = [mA, mB]

    def qk_chunk(qb, h, hh, par, kc, m8):
        g = h // HPG if isinstance(h, int) else lax.shift_right_logical(h, 2)
        kk = ld(r_s[G + g, kc * tk // 2:(kc + 1) * tk // 2, :])
        parts = []
        if hh > 0:
            parts.append(jnp.zeros((hh * DH // 2, tq), u32))
        parts.append(t_s[g, qb, hh * DH // 2:(hh + 1) * DH // 2, :])
        if hh < HPG - 1:
            parts.append(jnp.zeros(((HPG - 1 - hh) * DH // 2, tq), u32))
        qm = ld(jnp.concatenate(parts, axis=0))
        s = jnp.dot(kk, qm, preferred_element_type=f32)
        sbuf[par][kc * tk:(kc + 1) * tk, :] = s
        mc = jnp.max(s.reshape(tk // 8, 8, tq), axis=0)
        m8 = mc if m8 is None else jnp.maximum(m8, mc)
        if kc == nkc - 1:
            mbuf[par][...] = jnp.max(m8, axis=0, keepdims=True)
        return m8

    transpose_tiles(nq - 1, NC - 1)
    m8 = None
    for kc in range(nkc):
        m8 = qk_chunk(0, 0, 0, 0, kc, m8)
    m8 = None
    for kc in range(d):
        m8 = qk_chunk(0, 1, 1, 1, kc, m8)
    m8_s[...] = m8

    def flush_o(jprev):
        for gi in range(GPI):
            o_s[jprev * GPI + gi] = st(
                otg_s[gi * 128:(gi + 1) * 128, :].T.astype(bf16))

    def block(qb, carry):
        niter = H // _UNROLL

        def body(j, c):
            h0 = j * _UNROLL
            flush_o(jnp.maximum(j - 1, 0))
            m8 = m8_s[...]
            m_hist = []
            for u in range(_UNROLL):
                par = u % 2
                g = j * GPI + u // HPG
                hh = u % HPG
                m = jnp.broadcast_to(mbuf[par][...], (8, tq))
                acc = z_s[...]
                l8 = None
                for kc in range(nkc):
                    me = m
                    if len(m_hist) >= _MLAG:
                        mm = m_hist[-_MLAG]
                        me = me + jnp.where(mm == mm, 0.0, mm)
                    p = jnp.exp2(sbuf[par][kc * tk:(kc + 1) * tk, :]
                                 .reshape(tk // 8, 8, tq) - me)
                    for i in reversed(range(tk // 8)):
                        l8 = p[i] if l8 is None else l8 + p[i]
                    pb = p.reshape(tk, tq).astype(bf16)
                    tt = u * nkc + kc + nkc + d
                    un, kn = tt // nkc, tt % nkc
                    if kn == 0:
                        m8 = None
                    hn = h0 + un
                    if un < _UNROLL:
                        qbn, hn_ = qb, hn
                    else:
                        wrap = (hn >= H).astype(jnp.int32)
                        qbn = jnp.minimum(qb + wrap, nq - 1)
                        hn_ = hn - wrap * H
                    m8 = qk_chunk(qbn, hn_, un % HPG, un % 2, kn, m8)
                    m_hist.append(m8)
                    vt = ld(t_s[2 * G + g, kc // cpb, hh * DH // 2:(hh + 1) * DH // 2,
                                (kc % cpb) * tk:(kc % cpb + 1) * tk])
                    acc = acc + jnp.dot(vt, pb, preferred_element_type=f32)
                l = jnp.sum(l8, axis=0, keepdims=True)
                otg_s[u * DH:(u + 1) * DH, :] = acc * (1.0 / l)
            m8_s[...] = m8
            return c

        lax.fori_loop(0, niter, body, 0)

        @pl.when(qb == 0)
        def _():
            for cp in late_copies():
                cp.wait()
            b1_s[...] = b1r_s[...].astype(f32).reshape(1, F)
            b2_s[...] = b2r_s[...].astype(f32).reshape(1, D)

        @pl.when(qb > 0)
        def _():
            out_copy(qb - 1).wait()

        flush_o(niter - 1)
        xoff = pl.multiple_of(qb * tq, tq)
        w1c = w1_s[:, 0:_TF0]
        b1c = b1_s[:, 0:_TF0]
        npc = tq // _WOROWS
        hids = []

        def wo_piece(p):
            r0, r1 = p * _WOROWS, (p + 1) * _WOROWS
            o = jnp.concatenate([ld(o_s[g, r0 // 2:r1 // 2, :]) for g in range(G)], axis=1)
            hres = x_s[pl.ds(xoff + r0, _WOROWS), :].astype(f32) + jnp.dot(
                o, wo_s[...], preferred_element_type=f32)
            y_s[r0 // 2:r1 // 2, :] = st(_layernorm_twice(hres).astype(bf16))
            acc_s[r0:r1, :] = hres

        def m1_piece(p):
            r0, r1 = p * _WOROWS, (p + 1) * _WOROWS
            hid = jnp.dot(ld(y_s[r0 // 2:r1 // 2, :]), w1c, preferred_element_type=f32)
            hids.append(_gelu(hid + b1c).astype(bf16))

        for p in range(npc + _WOLAG):
            if p < npc:
                wo_piece(p)
            if p >= _WOLAG:
                m1_piece(p - _WOLAG)
        hid = jnp.concatenate(hids, axis=0)
        acc_s[...] = (acc_s[...] + jnp.dot(hid, w2_s[0:_TF0, :],
                                           preferred_element_type=f32)) + b2_s[...]

        def mlp(c, carry):
            foff = pl.multiple_of(_TF0 + c * _TF, 128)
            hid = jnp.dot(ld(y_s[...]), w1_s[:, pl.ds(foff, _TF)],
                          preferred_element_type=f32)
            hid = _gelu(hid + b1_s[:, pl.ds(foff, _TF)]).astype(bf16)
            a = acc_s[...] + jnp.dot(hid, w2_s[pl.ds(foff, _TF), :],
                                     preferred_element_type=f32)
            acc_s[...] = a
            out_s[...] = a.astype(out_s.dtype)
            return carry

        lax.fori_loop(0, (F - _TF0) // _TF, mlp, 0)
        out_copy(qb).start()
        return carry

    lax.fori_loop(0, nq, block, 0)
    out_copy(nq - 1).wait()


@jax.jit
def pallas_sequential_preLN__softmax_full_mha__mixer_channel_mlp__prompt_kernel(
    A_x: jax.Array,
    A_wqkv: jax.Array,
    A_wo: jax.Array,
    B_x: jax.Array,
    B_w1: jax.Array,
    B_b1: jax.Array,
    B_w2: jax.Array,
    B_b2: jax.Array,
):
    B, S, D = A_x.shape
    assert B == 1
    F = B_w1.shape[1]
    H, tq = _H, _TQ
    DH = D // H
    nq = S // tq
    G = D // 128
    assert S % tq == 0 and D % tq == 0 and (F - _TF0) % _TF == 0 and F > _TF0
    x = A_x.reshape(S, D)
    bf = jnp.bfloat16
    f32 = jnp.float32
    u32 = jnp.uint32
    hbm = pl.BlockSpec(memory_space=pl.ANY)

    out = pl.pallas_call(
        functools.partial(_kernel, S=S, D=D, F=F),
        in_specs=[hbm] * 7,
        out_specs=hbm,
        out_shape=jax.ShapeDtypeStruct((S, D), A_x.dtype),
        scratch_shapes=[
            pltpu.VMEM((S, D), bf),
            pltpu.VMEM((_NC, D, 3 * D // _NC), bf),
            pltpu.VMEM((D, D), bf),
            pltpu.VMEM((D, F), bf),
            pltpu.VMEM((F, D), bf),
            pltpu.VMEM((2, tq // 2, D), u32),
            pltpu.VMEM((3 * G, S // 2, 128), u32),
            pltpu.VMEM((3 * G, nq, 64, tq), u32),
            pltpu.VMEM((3 * D // _NC // 128, tq // 2, 128), u32),
            pltpu.VMEM((S, tq), f32),
            pltpu.VMEM((S, tq), f32),
            pltpu.VMEM((1, tq), f32),
            pltpu.VMEM((1, tq), f32),
            pltpu.VMEM((8, tq), f32),
            pltpu.VMEM((DH, tq), f32),
            pltpu.VMEM((_UNROLL * DH, tq), f32),
            pltpu.VMEM((G, tq // 2, 128), u32),
            pltpu.VMEM((tq // 2, D), u32),
            pltpu.VMEM((tq, D), f32),
            pltpu.VMEM((tq, D), bf),
            pltpu.VMEM((1, F), f32),
            pltpu.VMEM((1, D), f32),
            pltpu.VMEM((F,), bf),
            pltpu.VMEM((D,), bf),
            pltpu.SemaphoreType.DMA((3,)),
            pltpu.SemaphoreType.DMA((_NC,)),
            pltpu.SemaphoreType.DMA((_NW0,)),
            pltpu.SemaphoreType.DMA((_NC,)),
            pltpu.SemaphoreType.DMA((5,)),
            pltpu.SemaphoreType.DMA((1,)),
        ],
        compiler_params=pltpu.CompilerParams(
            vmem_limit_bytes=110 * 1024 * 1024,
        ),
    )(x, A_wqkv, A_wo, B_w1, B_b1, B_w2, B_b2)
    return out.reshape(B, S, D)
```
